```python
import jax
import jax.numpy as jnp

def _softmax(x, axis=-1):
    return jax.nn.softmax(x, axis=axis)
def _gelu(x):
    return jax.nn.gelu(x, approximate=True)
def _silu(x):
    return jax.nn.silu(x)
def _sigmoid(x):
    return jax.nn.sigmoid(x)
def _layernorm(x, axis=-1, eps=1e-5):
    m = jnp.mean(x, axis=axis, keepdims=True)
    v = jnp.var(x, axis=axis, keepdims=True)
    return (x - m) / jnp.sqrt(v + eps)
def _scatter_add(tgt, idx, src, axis=0):
    return tgt.at[idx].add(src)
def _segment_sum(src, seg, n):
    return jax.ops.segment_sum(src, seg, n)
class _Rng:
    def __init__(self, key):
        self._k = key
    def _next(self):
        self._k, sub = jax.random.split(self._k)
        return sub
    def normal(self, shape):
        return jax.random.normal(self._next(), shape, dtype=jnp.bfloat16)
    def randint(self, lo, hi, shape):
        return jax.random.randint(self._next(), shape, lo, hi, dtype=jnp.int32)
    def uniform(self, shape, lo=0.0, hi=1.0):
        return jax.random.uniform(self._next(), shape, jnp.bfloat16, lo, hi)
    def permutation(self, n):
        return jax.random.permutation(self._next(), n)


kernel_name = 'standalone__structured_sparse_n_m__ragged'

def setup_inputs():
    _rng = _Rng(jax.random.key(int.from_bytes(__import__("os").urandom(4), "little")))
    _w = (lambda a: (lambda t: t.astype(jnp.bfloat16) if jnp.issubdtype(t.dtype, jnp.floating) else t)(jnp.asarray(a)))
    B, S, D = 16, 4096, 576
    assert D % 4 == 0, "d_model must be divisible by M=4 for 2:4 sparsity"
    return {
        "x": _w((lambda *s: _rng.normal(s) * 0.05)(B, S, D)),
        "w": _w((lambda *s: _rng.normal(s) * 0.05)(D, D)),
        "b": _w((lambda *s: _rng.normal(s) * 0.05)(D)),
    }

def reference(x, w, b):
    B, S, D = x.shape
    N, M = 2, 4
    G = D // M
    wg = w.reshape(G, M, D)
    mag = jnp.abs(wg)
    order = jnp.argsort(mag, 1)
    thr = jnp.take_along_axis(mag, order[:, M - N:M - N + 1, :], 1)
    mask = (lambda x, dt: x.astype(dt))(mag >= thr, w.dtype)
    wp = (wg * mask).reshape(D, D)
    return jnp.einsum("bsd,df->bsf", x, wp) + b
```

```python
import jax
import jax.numpy as jnp
from jax import lax
import jax.experimental.pallas as pl
import jax.experimental.pallas.tpu as pltpu

F32, BF16, I32 = jnp.float32, jnp.bfloat16, jnp.int32

NU, UR = 9, 64
Q = 144
W = 512
NG = 4
NO = 80
SWITCH = 65
NSUB = 4

DEEP = ("R0", "K0", "R1", "K1")
SLOT = {"R0": 0, "K0": 7, "R1": 14, "K1": 21, "M1": 28, "N1": 30,
        "D00": 32, "D11": 35, "D01": 38, "D10": 41}
NA = 44


def _prune_packed(u):
    mate = lax.broadcasted_iota(I32, u.shape, 0) ^ 1
    lo = pltpu.bitcast((u << 16) & 0x7FFFFFFF, F32)
    hi = pltpu.bitcast(u & 0x7FFF0000, F32)
    big, small = jnp.maximum(lo, hi), jnp.minimum(lo, hi)
    nbig = jnp.take_along_axis(big, mate, axis=0, mode="promise_in_bounds")
    nsmall = jnp.take_along_axis(small, mate, axis=0, mode="promise_in_bounds")
    thr = jnp.maximum(jnp.minimum(big, nbig), jnp.maximum(small, nsmall))
    return u & (jnp.where(lo < thr, 0, 0xFFFF) | jnp.where(hi < thr, 0, -65536))


def _prune_rows(w_bf16):
    u = pltpu.bitcast(w_bf16, I32)
    return jnp.concatenate(
        [_prune_packed(u[8 * i:8 * i + 8]) for i in range(u.shape[0] // 8)], axis=0)


def _kernel(x_hbm, w_hbm, b_hbm, o_hbm,
            xbuf, obuf, wbuf, bbuf, a_ref, bias_ref, isem, osem, wsem):
    NB, _, _, S = x_hbm.shape
    D = NU * UR
    CPB = S // W
    NCH = NB * CPB

    def read_piece(b, j, c):
        rows = pl.ds(pl.multiple_of(8 * j, 8), 8)
        q = b * CPB + c
        return pltpu.make_async_copy(
            x_hbm.at[b, :, rows, pl.ds(c * W, W)], xbuf.at[q, :, rows, :], isem.at[q])

    def write_piece(b, j, c):
        rows = pl.ds(pl.multiple_of(8 * j, 8), 8)
        s = (b * CPB) % NO + c
        return pltpu.make_async_copy(
            obuf.at[s, :, rows, :], o_hbm.at[b, :, rows, pl.ds(c * W, W)], osem.at[s])

    def write_half_chunk(q, h):
        cols = pl.ds(pl.multiple_of((q % CPB) * W + h * (W // 2), W // 2), W // 2)
        return pltpu.make_async_copy(
            obuf.at[q % NO, :, :, pl.ds(h * (W // 2), W // 2)],
            o_hbm.at[q // CPB, :, :, cols], osem.at[q % NO])

    def wait_read(q):
        pltpu.make_async_copy(xbuf.at[q], xbuf.at[q], isem.at[q]).wait()

    def wait_write(s):
        pltpu.make_async_copy(obuf.at[s], obuf.at[s], osem.at[s]).wait()

    blocks = [(0, 128), (128, 128), (256, 128), (384, 128), (512, 64)]
    bcp = pltpu.make_async_copy(b_hbm, bbuf, wsem.at[len(blocks)])
    wcp = [pltpu.make_async_copy(w_hbm.at[pl.ds(o, n)], wbuf.at[pl.ds(o, n)], wsem.at[i])
           for i, (o, n) in enumerate(blocks)]
    bcp.start()
    for cp in wcp:
        cp.start()
    bcp.wait()
    for q in range(CPB):
        pltpu.make_async_copy(x_hbm.at[0, :, :, pl.ds(q * W, W)], xbuf.at[q], isem.at[q]).start()

    def quarters(t):
        t = t.reshape(NU, UR, 128)
        return [[t[:, 32 * i + 16 * r:32 * i + 16 * r + 16].reshape(Q, 128) for r in range(2)]
                for i in range(2)]

    wt = []
    for cp, (o, n) in zip(wcp, blocks):
        cp.wait()
        p = _prune_rows(wbuf[o:o + n, :])
        if n == 64:
            p = jnp.concatenate([p, p], axis=0)
        wt.append(quarters(pltpu.bitcast(p, BF16).T.astype(F32)))
    U1, U2, V1, V2, T = wt
    bias = quarters(jnp.broadcast_to(bbuf[...].reshape(1, D).astype(F32), (128, D)).T)
    for m in range(4):
        bias_ref[m] = bias[m // 2][m % 2]

    def put(name, tiles):
        for i, v in enumerate(tiles):
            a_ref[SLOT[name] + i] = v.astype(BF16)

    def add(a, b):
        return [p + q for p, q in zip(a, b)]

    def sub(a, b):
        return [p - q for p, q in zip(a, b)]

    for name, m, n in (("R0", add(U1[0], U2[0]), add(V1[0], V2[0])), ("K0", U2[1], V1[0]),
                       ("R1", add(U1[1], U2[1]), add(V1[1], V2[1])), ("K1", U1[0], V2[1])):
        put(name, [m[0] + n[1], m[1] + n[1], m[0], n[1], m[0] + n[0], m[1] - m[0], n[0] - n[1]])
    put("M1", add(U1[0], U2[1]))
    put("N1", add(V1[0], V2[1]))
    low = lax.broadcasted_iota(I32, (Q, 128), 1) < 64
    for name, g, t in (("D00", sub(U2[0], U2[1]), T[0]), ("D11", sub(U1[1], U1[0]), T[1]),
                       ("D01", sub(V2[0], V2[1]), T[0]), ("D10", sub(V1[1], V1[0]), T[1])):
        put(name, [jnp.where(low, g[1], t[0]), jnp.where(low, g[0] - g[1], g[0]),
                   jnp.where(low, t[1] - t[0], g[1])])

    def mm(i, k, rhs):
        lhs = a_ref[i] if k == 1 else a_ref[i:i + k].reshape(k * Q, 128)
        return jnp.dot(lhs, rhs.astype(BF16), preferred_element_type=F32)

    def compute_chunk(q, hook):
        s = q % NO
        cache = {}
        ticks = iter(range(12))

        def X(h, j, u):
            if (h, j, u) not in cache:
                lanes = pl.ds((2 * h + j) * 128, 128)
                v = (xbuf[q, 2 * u:2 * u + 2, :, lanes].reshape(128, 128) if u < 4
                     else xbuf[q, 8, :, lanes])
                cache[h, j, u] = v.astype(F32)
            return cache[h, j, u]

        def deep_rhs(name, h):
            if name == "R0":
                return X(h, 1, 1), X(h, 0, 3)
            if name == "R1":
                return X(h, 0, 0), X(h, 1, 2)
            if name == "K0":
                return X(h, 0, 1) - X(h, 0, 0), X(h, 0, 2) - X(h, 0, 3)
            return X(h, 1, 0) - X(h, 1, 1), X(h, 1, 3) - X(h, 1, 2)

        deep = {}
        for name in DEEP:
            (m0, n0), (m1, n1) = deep_rhs(name, 0), deep_rhs(name, 1)
            a = SLOT[name]
            p5 = mm(a + 4, 1, n1)
            p2 = mm(a + 1, 1, m0)
            p4 = mm(a + 3, 1, n0 - m0)
            p3 = mm(a + 2, 1, m1 - n1)
            if name[0] == "R":
                p5 = p5 + bias_ref[2 * int(name[1])]
                p2 = p2 + bias_ref[2 * int(name[1]) + 1]
            c01, c10, e00, e11 = p3 + p5, p2 + p4, p4 + p5, p2 + p3
            p1 = mm(a, 1, m0 - n1)
            p7 = mm(a + 6, 1, n0 - n1)
            p6 = mm(a + 5, 1, m1 - m0)
            deep[name, 0] = [e00 + p1 + p7, c10]
            deep[name, 1] = [c01, e11 - p1 + p6]
            hook(next(ticks))

        def shallow(name, g, t):
            a = SLOT[name]
            both = mm(a, 1, jnp.concatenate([g[:64], t], axis=0))
            return [both + mm(a + 1, 1, g),
                    both + mm(a + 2, 1, jnp.concatenate([t, g[64:]], axis=0))]

        for h in range(2):
            for name, j, u in (("M1", 0, 0), ("N1", 1, 2)):
                y = mm(SLOT[name], 2, X(h, j, u) - X(h, 1 - j, u + 1))
                y = [y[:Q], y[Q:]]
                for i, jj, uu in ((0, j, u + 1), (1, 1 - j, u)):
                    d = shallow("D%d%d" % (i, jj), X(h, jj, uu) - X(h, 1 - jj, uu), X(h, jj, 4))
                    for r in range(2):
                        v = deep["R%d" % i, h][r] + deep["K%d" % jj, h][r]
                        v = (v + y[r] if i == 0 else v - y[r]) + d[r]
                        obuf[s, :, pl.ds(32 * i + 16 * r, 16), pl.ds((2 * h + jj) * 128, 128)] = (
                            v.astype(BF16).reshape(NU, 16, 128))
                    hook(next(ticks))

    NPS = (NB - 1) * CPB // 2

    def start_dmas(q, part):
        ids = range(part * 2 * CPB // NSUB, (part + 1) * 2 * CPB // NSUB)

        @pl.when(q < NPS)
        def _():
            for i in ids:
                row = 2 * q + i // CPB
                read_piece(1 + row // 8, row % 8, i % CPB).start(priority=i % 2)

        qw = q - SWITCH
        if part == 0:
            @pl.when(qw == 0)
            def _():
                wait_read(NCH - 1)

        @pl.when((qw >= 0) & (qw < NPS))
        def _():
            for i in ids:
                row = 2 * qw + i // CPB
                write_piece(row // 8, row % 8, i % CPB).start()

        if part == 0:
            @pl.when(qw >= NPS)
            def _():
                for i in range(4):
                    write_half_chunk(2 * qw + i // 2, i % 2).start()

    def body(it, carry):
        for g in range(NG):
            q = it * NG + g

            @pl.when(q != NCH - 1)
            def _():
                wait_read(q)

            @pl.when(q >= NO)
            def _():
                wait_write(q - NO)

            def hook(k):
                if k % (12 // NSUB) == 0:
                    start_dmas(q, k // (12 // NSUB))

            compute_chunk(q, hook)
        return carry

    lax.fori_loop(0, NCH // NG, body, 0)
    for q in range(2 * (NCH - SWITCH), NCH):
        for h in range(2):
            write_half_chunk(q, h).start()
    for q in range(NCH - NO, NCH):
        wait_write(q % NO)


@jax.jit
def pallas_standalone__structured_sparse_n_m__ragged_kernel(
    x: jax.Array,
    w: jax.Array,
    b: jax.Array,
):
    B, S, D = x.shape
    xt = jnp.transpose(x, (0, 2, 1)).reshape(B, NU, UR, S)
    n_chunks = B * S // W
    out = pl.pallas_call(
        _kernel,
        in_specs=[pl.BlockSpec(memory_space=pl.ANY)] * 3,
        out_specs=pl.BlockSpec(memory_space=pl.ANY),
        out_shape=jax.ShapeDtypeStruct((B, NU, UR, S), x.dtype),
        scratch_shapes=[
            pltpu.VMEM((n_chunks, NU, UR, W), BF16),
            pltpu.VMEM((NO, NU, UR, W), BF16),
            pltpu.VMEM((D, D), BF16),
            pltpu.VMEM((D,), BF16),
            pltpu.VMEM((NA, Q, 128), BF16),
            pltpu.VMEM((4, Q, 128), F32),
            pltpu.SemaphoreType.DMA((n_chunks,)),
            pltpu.SemaphoreType.DMA((NO,)),
            pltpu.SemaphoreType.DMA((6,)),
        ],
        compiler_params=pltpu.CompilerParams(
            vmem_limit_bytes=127 * 1024 * 1024,
            disable_bounds_checks=True,
            disable_semaphore_checks=True,
            flags={"XLA_TPU_RESCHEDULE_DMA_DONES": True},
        ),
    )(xt, w, b)
    return jnp.transpose(out.reshape(B, D, S), (0, 2, 1))
```

```python
import jax
import jax.numpy as jnp
from jax import lax
import jax.experimental.pallas as pl
import jax.experimental.pallas.tpu as pltpu

F32, BF16, I32 = jnp.float32, jnp.bfloat16, jnp.int32

NU, UR = 9, 64
Q = 144
W = 512
NI = 10

READ_POINTS = (0, 3, 6, 9)
WRITE_POINTS = (3, 5, 7, 9)
WRITE_START = 25
WRITE_BURST = 4
WRITE_RATE = 30

SLOT = {"R0": 0, "R1": 7, "K0": 14, "K1": 21, "M1": 28, "N1": 30,
        "D00": 32, "D11": 35, "D01": 38, "D10": 41}
NA = 44


def _prune_packed(u):
    mate = lax.broadcasted_iota(I32, u.shape, 0) ^ 1
    lo = pltpu.bitcast((u << 16) & 0x7FFFFFFF, F32)
    hi = pltpu.bitcast(u & 0x7FFF0000, F32)
    big, small = jnp.maximum(lo, hi), jnp.minimum(lo, hi)
    nbig = jnp.take_along_axis(big, mate, axis=0, mode="promise_in_bounds")
    nsmall = jnp.take_along_axis(small, mate, axis=0, mode="promise_in_bounds")
    thr = jnp.maximum(jnp.minimum(big, nbig), jnp.maximum(small, nsmall))
    return u & (jnp.where(lo < thr, 0, 0xFFFF) | jnp.where(hi < thr, 0, -65536))


def _prune_rows(w_bf16):
    u = pltpu.bitcast(w_bf16, I32)
    return jnp.concatenate(
        [_prune_packed(u[8 * i:8 * i + 8]) for i in range(u.shape[0] // 8)], axis=0)


def _aligned(v, m):
    return v if isinstance(v, int) else pl.multiple_of(v, m)


def _select(cond, a, b):
    return (a if cond else b) if isinstance(cond, bool) else jnp.where(cond, a, b)


def _wait_until_filled(ref, sem):
    pltpu.make_async_copy(ref, ref, sem).wait()


def _kernel(x_hbm, w_hbm, b_hbm, o_hbm,
            xbuf, obuf, wbuf, bbuf, a_ref, bias_ref, xsem, osem, wsem):
    NB, _, _, S = x_hbm.shape
    D = NU * UR
    CPB = S // W

    def x_slot(b):
        return _select(b >= NI, b - NI, b) * CPB

    def read_piece(b, j, c, sem):
        rows = pl.ds(_aligned(8 * j, 8), 8)
        return pltpu.make_async_copy(
            x_hbm.at[b, :, rows, pl.ds(c * W, W)], xbuf.at[x_slot(b) + c, :, rows, :], sem)

    def write_group(r):
        last = r >= 16 * (NB - 1)
        return r >> 4, _select(last, r, r >> 1) & 7, (_select(last, r >> 3, r) & 1) * 4

    def start_writes(r):
        b, j, c0 = write_group(r)
        rows = pl.ds(_aligned(8 * j, 8), 8)
        for c in (c0, c0 + 1, c0 + 2, c0 + 3):
            pltpu.make_async_copy(
                obuf.at[b * CPB + c, :, rows, :],
                o_hbm.at[b, :, rows, pl.ds(_aligned(c * W, W), W)], osem.at[0]).start()

    blocks = [(0, 128), (128, 128), (256, 128), (384, 128), (512, 64)]
    wcp = [pltpu.make_async_copy(w_hbm.at[pl.ds(o, n)], wbuf.at[pl.ds(o, n)], wsem.at[i])
           for i, (o, n) in enumerate(blocks)]
    bcp = pltpu.make_async_copy(b_hbm, bbuf, wsem.at[len(blocks)])
    for cp in wcp:
        cp.start()
    bcp.start()

    @pl.loop(0, 2)
    def _(c):
        pltpu.make_async_copy(
            x_hbm.at[0, :, :, pl.ds(_aligned(c * W, W), W)], xbuf.at[c], xsem.at[c]).start()

    for lo, hi in ((2, 4), (4, CPB)):
        @pl.loop(0, 4)
        def _(j):
            for c in range(lo, hi):
                for k in range(2):
                    read_piece(0, 2 * j + k, c, xsem.at[c]).start(priority=k)

    def quarters(t):
        t = t.reshape(NU, UR, 128)
        return [[t[:, 32 * i + 16 * r:32 * i + 16 * r + 16].reshape(Q, 128) for r in range(2)]
                for i in range(2)]

    wt = []
    for cp, (o, n) in zip(wcp, blocks):
        cp.wait()
        p = _prune_rows(wbuf[o:o + n, :])
        if n == 64:
            p = jnp.concatenate([p, p], axis=0)
        wt.append(quarters(pltpu.bitcast(p, BF16).T.astype(F32)))
    U1, U2, V1, V2, T = wt
    bcp.wait()
    bias = quarters(jnp.broadcast_to(bbuf[...].reshape(1, D).astype(F32), (128, D)).T)
    for m in range(4):
        bias_ref[m] = bias[m // 2][m % 2]

    def put(name, tiles):
        for i, v in enumerate(tiles):
            a_ref[SLOT[name] + i] = v.astype(BF16)

    def add(a, b):
        return [p + q for p, q in zip(a, b)]

    def sub(a, b):
        return [p - q for p, q in zip(a, b)]

    for name, m, n in (("R0", add(U1[0], U2[0]), add(V1[0], V2[0])),
                       ("R1", add(U1[1], U2[1]), add(V1[1], V2[1])),
                       ("K0", U2[1], V1[0]), ("K1", U1[0], V2[1])):
        put(name, [m[0] + n[1], m[1] + n[1], m[0], n[1], m[0] + n[0], m[1] - m[0], n[0] - n[1]])
    put("M1", add(U1[0], U2[1]))
    put("N1", add(V1[0], V2[1]))
    low = lax.broadcasted_iota(I32, (Q, 128), 1) < 64
    for name, g, t in (("D00", sub(U2[0], U2[1]), T[0]), ("D11", sub(U1[1], U1[0]), T[1]),
                       ("D01", sub(V2[0], V2[1]), T[0]), ("D10", sub(V1[1], V1[0]), T[1])):
        put(name, [jnp.where(low, g[1], t[0]), jnp.where(low, g[0] - g[1], g[0]),
                   jnp.where(low, t[1] - t[0], g[1])])

    a_words = a_ref.bitcast(I32)

    def mm(i, k, rhs):
        lhs = a_words[i] if k == 1 else a_words[i:i + k].reshape(k * Q // 2, 128)
        return jnp.dot(pltpu.bitcast(lhs, BF16), rhs.astype(BF16), preferred_element_type=F32)

    def compute_chunk(b, c, at_point):
        s = x_slot(b) + c
        cache = {}
        points = iter(range(12))

        def X(h, j, u):
            if (h, j, u) not in cache:
                lanes = pl.ds((2 * h + j) * 128, 128)
                v = (xbuf[s, 2 * u:2 * u + 2, :, lanes].reshape(128, 128) if u < 4
                     else xbuf[s, 8, :, lanes])
                cache[h, j, u] = v.astype(F32)
            return cache[h, j, u]

        def deep_rhs(name, h):
            if name == "R0":
                return X(h, 1, 1), X(h, 0, 3)
            if name == "R1":
                return X(h, 0, 0), X(h, 1, 2)
            if name == "K0":
                return X(h, 0, 1) - X(h, 0, 0), X(h, 0, 2) - X(h, 0, 3)
            return X(h, 1, 0) - X(h, 1, 1), X(h, 1, 3) - X(h, 1, 2)

        deep = {}
        for name, h in (("R0", 0), ("R1", 0), ("K0", 1), ("K1", 1)):
            (m0, n0), (m1, n1) = deep_rhs(name, h), deep_rhs(name, 1 - h)
            a = SLOT[name]
            p5 = mm(a + 4, 1, n1)
            p2 = mm(a + 1, 1, m0)
            p4 = mm(a + 3, 1, n0 - m0)
            p3 = mm(a + 2, 1, m1 - n1)
            if name[0] == "R":
                p5 = p5 + bias_ref[2 * int(name[1])]
                p2 = p2 + bias_ref[2 * int(name[1]) + 1]
            c01, c10, e00, e11 = p3 + p5, p2 + p4, p4 + p5, p2 + p3
            p1 = mm(a, 1, m0 - n1)
            p7 = mm(a + 6, 1, n0 - n1)
            p6 = mm(a + 5, 1, m1 - m0)
            deep[name, h] = [e00 + p1 + p7, c10]
            deep[name, 1 - h] = [c01, e11 - p1 + p6]
            at_point(next(points))

        def shallow(name, g, t):
            a = SLOT[name]
            both = mm(a, 1, jnp.concatenate([g[:64], t], axis=0))
            return [both + mm(a + 1, 1, g),
                    both + mm(a + 2, 1, jnp.concatenate([t, g[64:]], axis=0))]

        for h in range(2):
            for name, j, u in (("M1", 0, 0), ("N1", 1, 2)):
                y = mm(SLOT[name], 2, X(h, j, u) - X(h, 1 - j, u + 1))
                y = [y[:Q], y[Q:]]
                for i, jj, uu in ((0, j, u + 1), (1, 1 - j, u)):
                    d = shallow("D%d%d" % (i, jj), X(h, jj, uu) - X(h, 1 - jj, uu), X(h, jj, 4))
                    for r in range(2):
                        v = deep["R%d" % i, h][r] + deep["K%d" % jj, h][r]
                        v = (v + y[r] if i == 0 else v - y[r]) + d[r]
                        obuf[b * CPB + c, :, pl.ds(32 * i + 16 * r, 16),
                             pl.ds((2 * h + jj) * 128, 128)] = v.astype(BF16).reshape(NU, 16, 128)
                    at_point(next(points))

    n_points = CPB * len(WRITE_POINTS)
    b_start = NB // 2 - 1

    def first_group(b, t):
        return (b * WRITE_RATE + (WRITE_BURST - b_start * WRITE_RATE + WRITE_RATE * t // n_points
                                  - WRITE_RATE * WRITE_START // n_points))

    def computed(r, b, c):
        rb, _, rc = write_group(r)
        return rb * CPB + rc + 3 < b * CPB + c

    assert computed(WRITE_BURST, b_start, 0)
    n_in_loop = min([first_group(NB, 0), 16 * NB] + [
        r for b in range(NB) for t in range(n_points)
        for r in range(first_group(b, t), first_group(b, t + 1))
        if r >= WRITE_BURST and not computed(r, b, t // len(WRITE_POINTS))])

    def start_dmas(b, c, point):
        if point in READ_POINTS:
            ahead, i0 = divmod(16 * c + 4 * READ_POINTS.index(point), 64)
            nb = 2 * b + (1 + ahead)

            @pl.when(nb < NB)
            def _():
                for i in range(i0, i0 + 4):
                    read_piece(nb, 2 * (i >> 4) + (i & 1), (i >> 1) & 7,
                               xsem.at[CPB - 1 + nb]).start(priority=i & 1)

        if point in WRITE_POINTS:
            t = c * len(WRITE_POINTS) + WRITE_POINTS.index(point)
            for r in range(WRITE_BURST if t == WRITE_START else 0):
                @pl.when(b == b_start)
                def _():
                    start_writes(r)

            for k in range(first_group(0, t + 1) - first_group(0, t)):
                r = first_group(b, t) + k

                @pl.when((r >= WRITE_BURST) & (r < n_in_loop))
                def _():
                    start_writes(r)

    @pl.loop(0, NB)
    def _(b):
        @pl.when(b > 0)
        def _():
            _wait_until_filled(xbuf.at[pl.ds(x_slot(b), CPB)], xsem.at[CPB - 1 + b])

        for c in range(CPB):
            @pl.when(b == 0)
            def _():
                _wait_until_filled(xbuf.at[c], xsem.at[c])

            compute_chunk(b, c, lambda point: start_dmas(b, c, point))

    for r in range(n_in_loop, 16 * NB):
        start_writes(r)
    _wait_until_filled(obuf, osem.at[0])


@jax.jit
def pallas_standalone__structured_sparse_n_m__ragged_kernel(
    x: jax.Array,
    w: jax.Array,
    b: jax.Array,
):
    B, S, D = x.shape
    assert (B, S, D) == (16, 8 * W, NU * UR)
    xt = jnp.transpose(x, (0, 2, 1)).reshape(B, NU, UR, S)
    out = pl.pallas_call(
        _kernel,
        in_specs=[pl.BlockSpec(memory_space=pl.ANY)] * 3,
        out_specs=pl.BlockSpec(memory_space=pl.ANY),
        out_shape=jax.ShapeDtypeStruct((B, NU, UR, S), x.dtype),
        scratch_shapes=[
            pltpu.VMEM((NI * S // W, NU, UR, W), BF16),
            pltpu.VMEM((B * S // W, NU, UR, W), BF16),
            pltpu.VMEM((D, D), BF16),
            pltpu.VMEM((D,), BF16),
            pltpu.VMEM((NA, Q, 128), BF16),
            pltpu.VMEM((4, Q, 128), F32),
            pltpu.SemaphoreType.DMA((S // W + B - 1,)),
            pltpu.SemaphoreType.DMA((1,)),
            pltpu.SemaphoreType.DMA((6,)),
        ],
        compiler_params=pltpu.CompilerParams(
            vmem_limit_bytes=127 * 1024 * 1024,
            disable_bounds_checks=True,
            disable_semaphore_checks=True,
            flags={"XLA_TPU_RESCHEDULE_DMA_DONES": True},
        ),
    )(xt, w, b)
    return jnp.transpose(out.reshape(B, D, S), (0, 2, 1))
```

```python
import jax
import jax.numpy as jnp
from jax import lax
import jax.experimental.pallas as pl
import jax.experimental.pallas.tpu as pltpu

F32, BF16, I32 = jnp.float32, jnp.bfloat16, jnp.int32

NU, UR = 9, 64
Q = 144
W = 512
NI = 10

READ_POINTS = (0, 3, 6, 9)
WRITE_POINTS = (3, 5, 7, 9)
WRITE_START = 25
WRITE_BURST = 4
WRITE_RATE = 30

SLOT = {"R0": 0, "R1": 7, "K0": 14, "K1": 21, "M1": 28, "N1": 30,
        "D00": 32, "D11": 35, "D01": 38, "D10": 41}
NA = 44


def _prune_packed(u):
    mate = lax.broadcasted_iota(I32, u.shape, 0) ^ 1
    lo = pltpu.bitcast((u << 16) & 0x7FFFFFFF, F32)
    hi = pltpu.bitcast(u & 0x7FFF0000, F32)
    big, small = jnp.maximum(lo, hi), jnp.minimum(lo, hi)
    nbig = jnp.take_along_axis(big, mate, axis=0, mode="promise_in_bounds")
    nsmall = jnp.take_along_axis(small, mate, axis=0, mode="promise_in_bounds")
    thr = jnp.maximum(jnp.minimum(big, nbig), jnp.maximum(small, nsmall))
    return u & (jnp.where(lo < thr, 0, 0xFFFF) | jnp.where(hi < thr, 0, -65536))


def _prune_rows(w_bf16):
    u = pltpu.bitcast(w_bf16, I32)
    return jnp.concatenate(
        [_prune_packed(u[8 * i:8 * i + 8]) for i in range(u.shape[0] // 8)], axis=0)


def _aligned(v, m):
    return v if isinstance(v, int) else pl.multiple_of(v, m)


def _select(cond, a, b):
    return (a if cond else b) if isinstance(cond, bool) else jnp.where(cond, a, b)


def _wait_until_filled(ref, sem):
    pltpu.make_async_copy(ref, ref, sem).wait()


def _kernel(x_hbm, w_hbm, b_hbm, o_hbm,
            xbuf, obuf, wbuf, bbuf, a_ref, bias_ref, xsem, osem, wsem):
    NB, _, _, S = x_hbm.shape
    D = NU * UR
    CPB = S // W

    def x_slot(b):
        return _select(b >= NI, b - NI, b) * CPB

    def read_piece(b, j, c, sem):
        rows = pl.ds(_aligned(8 * j, 8), 8)
        return pltpu.make_async_copy(
            x_hbm.at[b, :, rows, pl.ds(c * W, W)], xbuf.at[x_slot(b) + c, :, rows, :], sem)

    def write_group(r):
        last = r >= 16 * (NB - 1)
        return r >> 4, _select(last, r, r >> 1) & 7, (_select(last, r >> 3, r) & 1) * 4

    def start_writes(r):
        b, j, c0 = write_group(r)
        rows = pl.ds(_aligned(8 * j, 8), 8)
        for c in (c0, c0 + 1, c0 + 2, c0 + 3):
            pltpu.make_async_copy(
                obuf.at[b * CPB + c, :, rows, :],
                o_hbm.at[b, :, rows, pl.ds(_aligned(c * W, W), W)], osem.at[0]).start()

    blocks = [(0, 128), (128, 128), (256, 128), (384, 128), (512, 64)]
    wcp = [pltpu.make_async_copy(w_hbm.at[pl.ds(o, n)], wbuf.at[pl.ds(o, n)], wsem.at[i])
           for i, (o, n) in enumerate(blocks)]
    bcp = pltpu.make_async_copy(b_hbm, bbuf, wsem.at[len(blocks)])
    for cp in wcp:
        cp.start()
    bcp.start()

    @pl.loop(0, 2)
    def _(c):
        pltpu.make_async_copy(
            x_hbm.at[0, :, :, pl.ds(_aligned(c * W, W), W)], xbuf.at[c], xsem.at[c]).start()

    for lo, hi in ((2, 4), (4, CPB)):
        @pl.loop(0, 4)
        def _(j):
            for c in range(lo, hi):
                for k in range(2):
                    read_piece(0, 2 * j + k, c, xsem.at[c]).start(priority=k)

    def quarters(t):
        t = t.reshape(NU, UR, 128)
        return [[t[:, 32 * i + 16 * r:32 * i + 16 * r + 16].reshape(Q, 128) for r in range(2)]
                for i in range(2)]

    wt = []
    for cp, (o, n) in zip(wcp, blocks):
        cp.wait()
        p = _prune_rows(wbuf[o:o + n, :])
        if n == 64:
            p = jnp.concatenate([p, p], axis=0)
        wt.append(quarters(pltpu.bitcast(p, BF16).T.astype(F32)))
    U1, U2, V1, V2, T = wt
    bcp.wait()
    bias = quarters(jnp.broadcast_to(bbuf[...].reshape(1, D).astype(F32), (128, D)).T)
    for m in range(4):
        bias_ref[m] = bias[m // 2][m % 2]

    def put(name, tiles):
        for i, v in enumerate(tiles):
            a_ref[SLOT[name] + i] = pltpu.bitcast(v.astype(BF16), I32)

    def add(a, b):
        return [p + q for p, q in zip(a, b)]

    def sub(a, b):
        return [p - q for p, q in zip(a, b)]

    for name, m, n in (("R0", add(U1[0], U2[0]), add(V1[0], V2[0])),
                       ("R1", add(U1[1], U2[1]), add(V1[1], V2[1])),
                       ("K0", U2[1], V1[0]), ("K1", U1[0], V2[1])):
        put(name, [m[0] + n[1], m[1] + n[1], m[0], n[1], m[0] + n[0], m[1] - m[0], n[0] - n[1]])
    put("M1", add(U1[0], U2[1]))
    put("N1", add(V1[0], V2[1]))
    low = lax.broadcasted_iota(I32, (Q, 128), 1) < 64
    for name, g, t in (("D00", sub(U2[0], U2[1]), T[0]), ("D11", sub(U1[1], U1[0]), T[1]),
                       ("D01", sub(V2[0], V2[1]), T[0]), ("D10", sub(V1[1], V1[0]), T[1])):
        put(name, [jnp.where(low, g[1], t[0]), jnp.where(low, g[0] - g[1], g[0]),
                   jnp.where(low, t[1] - t[0], g[1])])

    def mm(i, k, rhs):
        lhs = a_ref[i] if k == 1 else a_ref[i:i + k].reshape(k * Q // 2, 128)
        return jnp.dot(pltpu.bitcast(lhs, BF16), rhs.astype(BF16), preferred_element_type=F32)

    def compute_chunk(b, c, at_point):
        s = x_slot(b) + c
        cache = {}
        points = iter(range(12))

        def X(h, j, u):
            if (h, j, u) not in cache:
                lanes = pl.ds((2 * h + j) * 128, 128)
                v = (xbuf[s, 2 * u:2 * u + 2, :, lanes].reshape(128, 128) if u < 4
                     else xbuf[s, 8, :, lanes])
                cache[h, j, u] = v.astype(F32)
            return cache[h, j, u]

        def deep_rhs(name, h):
            if name == "R0":
                return X(h, 1, 1), X(h, 0, 3)
            if name == "R1":
                return X(h, 0, 0), X(h, 1, 2)
            if name == "K0":
                return X(h, 0, 1) - X(h, 0, 0), X(h, 0, 2) - X(h, 0, 3)
            return X(h, 1, 0) - X(h, 1, 1), X(h, 1, 3) - X(h, 1, 2)

        deep = {}
        for name, h in (("R0", 0), ("R1", 0), ("K0", 1), ("K1", 1)):
            (m0, n0), (m1, n1) = deep_rhs(name, h), deep_rhs(name, 1 - h)
            a = SLOT[name]
            p5 = mm(a + 4, 1, n1)
            p2 = mm(a + 1, 1, m0)
            p4 = mm(a + 3, 1, n0 - m0)
            p3 = mm(a + 2, 1, m1 - n1)
            if name[0] == "R":
                p5 = p5 + bias_ref[2 * int(name[1])]
                p2 = p2 + bias_ref[2 * int(name[1]) + 1]
            c01, c10, e00, e11 = p3 + p5, p2 + p4, p4 + p5, p2 + p3
            p1 = mm(a, 1, m0 - n1)
            p7 = mm(a + 6, 1, n0 - n1)
            p6 = mm(a + 5, 1, m1 - m0)
            deep[name, h] = [e00 + p1 + p7, c10]
            deep[name, 1 - h] = [c01, e11 - p1 + p6]
            at_point(next(points))

        def shallow(name, g, t):
            a = SLOT[name]
            both = mm(a, 1, jnp.concatenate([g[:64], t], axis=0))
            return [both + mm(a + 1, 1, g),
                    both + mm(a + 2, 1, jnp.concatenate([t, g[64:]], axis=0))]

        for h in range(2):
            for name, j, u in (("M1", 0, 0), ("N1", 1, 2)):
                y = mm(SLOT[name], 2, X(h, j, u) - X(h, 1 - j, u + 1))
                y = [y[:Q], y[Q:]]
                for i, jj, uu in ((0, j, u + 1), (1, 1 - j, u)):
                    d = shallow("D%d%d" % (i, jj), X(h, jj, uu) - X(h, 1 - jj, uu), X(h, jj, 4))
                    for r in range(2):
                        v = deep["R%d" % i, h][r] + deep["K%d" % jj, h][r]
                        v = (v + y[r] if i == 0 else v - y[r]) + d[r]
                        obuf[b * CPB + c, :, pl.ds(32 * i + 16 * r, 16),
                             pl.ds((2 * h + jj) * 128, 128)] = v.astype(BF16).reshape(NU, 16, 128)
                    at_point(next(points))

    n_points = CPB * len(WRITE_POINTS)
    b_start = NB // 2 - 1

    def first_group(b, t):
        return (b * WRITE_RATE + (WRITE_BURST - b_start * WRITE_RATE + WRITE_RATE * t // n_points
                                  - WRITE_RATE * WRITE_START // n_points))

    def computed(r, b, c):
        rb, _, rc = write_group(r)
        return rb * CPB + rc + 3 < b * CPB + c

    assert computed(WRITE_BURST, b_start, 0)
    n_in_loop = min([first_group(NB, 0), 16 * NB] + [
        r for b in range(NB) for t in range(n_points)
        for r in range(first_group(b, t), first_group(b, t + 1))
        if r >= WRITE_BURST and not computed(r, b, t // len(WRITE_POINTS))])

    def start_dmas(b, c, point):
        if point in READ_POINTS:
            ahead, i0 = divmod(16 * c + 4 * READ_POINTS.index(point), 64)
            nb = 2 * b + (1 + ahead)

            @pl.when(nb < NB)
            def _():
                for i in range(i0, i0 + 4):
                    read_piece(nb, 2 * (i >> 4) + (i & 1), (i >> 1) & 7,
                               xsem.at[CPB - 1 + nb]).start(priority=i & 1)

        if point in WRITE_POINTS:
            t = c * len(WRITE_POINTS) + WRITE_POINTS.index(point)
            for r in range(WRITE_BURST if t == WRITE_START else 0):
                @pl.when(b == b_start)
                def _():
                    start_writes(r)

            for k in range(first_group(0, t + 1) - first_group(0, t)):
                r = first_group(b, t) + k

                @pl.when((r >= WRITE_BURST) & (r < n_in_loop))
                def _():
                    start_writes(r)

    @pl.loop(0, NB)
    def _(b):
        @pl.when(b > 0)
        def _():
            _wait_until_filled(xbuf.at[pl.ds(x_slot(b), CPB)], xsem.at[CPB - 1 + b])

        for c in range(CPB):
            @pl.when(b == 0)
            def _():
                _wait_until_filled(xbuf.at[c], xsem.at[c])

            compute_chunk(b, c, lambda point: start_dmas(b, c, point))

    for r in range(n_in_loop, 16 * NB):
        start_writes(r)
    _wait_until_filled(obuf, osem.at[0])


@jax.jit
def pallas_standalone__structured_sparse_n_m__ragged_kernel(
    x: jax.Array,
    w: jax.Array,
    b: jax.Array,
):
    B, S, D = x.shape
    assert (B, S, D) == (16, 8 * W, NU * UR)
    xt = jnp.transpose(x, (0, 2, 1)).reshape(B, NU, UR, S)
    out = pl.pallas_call(
        _kernel,
        in_specs=[pl.BlockSpec(memory_space=pl.ANY)] * 3,
        out_specs=pl.BlockSpec(memory_space=pl.ANY),
        out_shape=jax.ShapeDtypeStruct((B, NU, UR, S), x.dtype),
        scratch_shapes=[
            pltpu.VMEM((NI * S // W, NU, UR, W), BF16),
            pltpu.VMEM((B * S // W, NU, UR, W), BF16),
            pltpu.VMEM((D, D), BF16),
            pltpu.VMEM((D,), BF16),
            pltpu.VMEM((NA, Q // 2, 128), I32),
            pltpu.VMEM((4, Q, 128), F32),
            pltpu.SemaphoreType.DMA((S // W + B - 1,)),
            pltpu.SemaphoreType.DMA((1,)),
            pltpu.SemaphoreType.DMA((6,)),
        ],
        compiler_params=pltpu.CompilerParams(
            vmem_limit_bytes=127 * 1024 * 1024,
            disable_bounds_checks=True,
            disable_semaphore_checks=True,
            flags={"XLA_TPU_RESCHEDULE_DMA_DONES": True},
        ),
    )(xt, w, b)
    return jnp.transpose(out.reshape(B, D, S), (0, 2, 1))
```

```python
import jax
import jax.numpy as jnp
from jax import lax
import jax.experimental.pallas as pl
import jax.experimental.pallas.tpu as pltpu

F32, BF16, I32 = jnp.float32, jnp.bfloat16, jnp.int32

NU, UR = 9, 64
Q = 144
W = 512
NI = 5

READ_POINTS = (0, 3, 6, 9)
WRITE_POINTS = (3, 5, 7, 9)
READ_SPLIT = 2
WRITE_START = 25
WRITE_BURST = 2
WRITE_RATE = 15
WRITE_LAST = (6, 7, 9, 11, 13, 15, 17, 19, 21, 23, 25, 27)

SLOT = {"R0": 0, "R1": 7, "K0": 14, "K1": 21, "M1": 28, "N1": 30,
        "D00": 32, "D11": 35, "D01": 38, "D10": 41}
NA = 44


def _prune_packed(u):
    mate = lax.broadcasted_iota(I32, u.shape, 0) ^ 1
    lo = pltpu.bitcast((u << 16) & 0x7FFFFFFF, F32)
    hi = pltpu.bitcast(u & 0x7FFF0000, F32)
    big, small = jnp.maximum(lo, hi), jnp.minimum(lo, hi)
    nbig = jnp.take_along_axis(big, mate, axis=0, mode="promise_in_bounds")
    nsmall = jnp.take_along_axis(small, mate, axis=0, mode="promise_in_bounds")
    thr = jnp.maximum(jnp.minimum(big, nbig), jnp.maximum(small, nsmall))
    return u & (jnp.where(lo < thr, 0, 0xFFFF) | jnp.where(hi < thr, 0, -65536))


def _prune_rows(w_bf16):
    u = pltpu.bitcast(w_bf16, I32)
    return jnp.concatenate(
        [_prune_packed(u[8 * i:8 * i + 8]) for i in range(u.shape[0] // 8)], axis=0)


def _rows(j):
    return pl.ds(8 * j if isinstance(j, int) else pl.multiple_of(8 * j, 8), 8)


def _wait_until_filled(ref, sem):
    pltpu.make_async_copy(ref, ref, sem).wait()


def _kernel(x_hbm, w_hbm, b_hbm, o_hbm,
            xbuf, obuf, wbuf, bbuf, a_ref, bias_ref, xsem, osem, wsem):
    NP = x_hbm.shape[0]
    D = NU * UR

    def x_slot(k):
        return k if isinstance(k, int) else jnp.where(k >= NI, k - NI, k)

    def start_read(k, j, c, sem, queue, lo=0, hi=NU):
        pltpu.make_async_copy(
            x_hbm.at[k, lo:hi, _rows(j), pl.ds(c * W, W)],
            xbuf.at[x_slot(k), c, lo:hi, _rows(j), :], sem).start(priority=queue)

    def start_write(k, j, c2):
        pltpu.make_async_copy(
            obuf.at[k, c2, :, _rows(j), :],
            o_hbm.at[k, :, _rows(j), pl.ds(c2 * 2 * W, 2 * W)], osem.at[0]).start()

    def start_row_group(r):
        for c2 in range(4):
            start_write(r >> 4, r & 15, c2)

    def start_last_group(r):
        for i in range(4):
            if r < 8:
                start_write(NP - 1, 2 * r + i // 2, i % 2)
            else:
                start_write(NP - 1, 8 * (r & 1) + 2 * i + ((r >> 1) & 1), r // 4)

    blocks = [(0, 2), (2, 2), (4, 2), (6, 2), (8, 1)]
    wcp = [pltpu.make_async_copy(
        w_hbm.at[pl.ds(UR * o, UR * n)], wbuf.at[pl.ds(UR * o, UR * n)], wsem.at[i])
        for i, (o, n) in enumerate(blocks)]
    bcp = pltpu.make_async_copy(b_hbm, bbuf, wsem.at[len(blocks)])
    for cp in wcp:
        cp.start()
    bcp.start()

    @pl.loop(0, 3)
    def _(i):
        pltpu.make_async_copy(x_hbm.at[0, pl.ds(3 * i, 3), :, pl.ds(0, W)],
                              xbuf.at[0, 0, pl.ds(3 * i, 3)], xsem.at[0]).start()

    for lo, hi in ((1, 2), (2, 4)):
        @pl.loop(0, 8)
        def _(j):
            for c in range(lo, hi):
                for i in range(2):
                    start_read(0, 2 * j + i, c, xsem.at[c], i)

    def quarters(t):
        return [[jnp.concatenate([t[UR * n + o:UR * n + o + 16] for n in (0, 2, 4, 6, 8, 1, 3, 5, 7)])
                 for o in (32 * i, 32 * i + 16)] for i in range(2)]

    wp = []
    for cp, (o, n) in zip(wcp, blocks):
        cp.wait()
        wp += [_prune_rows(wbuf[UR * i:UR * (i + 1), :]) for i in range(o, o + n)]
    U1, V1, U2, V2, T = [
        quarters(pltpu.bitcast(jnp.concatenate([wp[i], wp[j]]), BF16).T.astype(F32))
        for i, j in ((0, 2), (1, 3), (4, 6), (5, 7), (8, 8))]
    bcp.wait()
    bias = quarters(jnp.broadcast_to(bbuf[...].reshape(1, D).astype(F32), (128, D)).T)
    for m in range(4):
        bias_ref[m] = bias[m // 2][m % 2]

    def put(name, tiles):
        for i, v in enumerate(tiles):
            a_ref[SLOT[name] + i] = pltpu.bitcast(v.astype(BF16), I32)

    def add(a, b):
        return [p + q for p, q in zip(a, b)]

    def sub(a, b):
        return [p - q for p, q in zip(a, b)]

    for name, m, n in (("R0", add(U1[0], U2[0]), add(V1[0], V2[0])),
                       ("R1", add(U1[1], U2[1]), add(V1[1], V2[1])),
                       ("K0", U2[1], V1[0]), ("K1", U1[0], V2[1])):
        put(name, [m[0] + n[1], m[1] + n[1], m[0], n[1], m[0] + n[0], m[1] - m[0], n[0] - n[1]])
    put("M1", add(U1[0], U2[1]))
    put("N1", add(V1[0], V2[1]))
    low = lax.broadcasted_iota(I32, (Q, 128), 1) < 64
    for name, g, t in (("D00", sub(U2[0], U2[1]), T[0]), ("D11", sub(U1[1], U1[0]), T[1]),
                       ("D01", sub(V2[0], V2[1]), T[0]), ("D10", sub(V1[1], V1[0]), T[1])):
        put(name, [jnp.where(low, g[1], t[0]), jnp.where(low, g[0] - g[1], g[0]),
                   jnp.where(low, t[1] - t[0], g[1])])

    def mm(i, n, rhs):
        lhs = a_ref[i] if n == 1 else a_ref[i:i + n].reshape(n * Q // 2, 128)
        return jnp.dot(pltpu.bitcast(lhs, BF16), rhs.astype(BF16), preferred_element_type=F32)

    def compute_chunk(k, half, c, e, at_point):
        slot, col = x_slot(k), 4 * half + c
        cache = {}
        points = iter(range(12))

        def X(h, j, u):
            if (h, j, u) not in cache:
                g, o = divmod(NU * e + (0, 4, 1, 5, 8)[u], 2)
                v = xbuf[slot, col, g:g + (2 if u < 4 else 1), pl.ds(UR * o, UR),
                         pl.ds((2 * h + j) * 128, 128)]
                cache[h, j, u] = v.reshape(-1, 128).astype(F32)
            return cache[h, j, u]

        def deep_rhs(name, h):
            if name == "R0":
                return X(h, 1, 1), X(h, 0, 3)
            if name == "R1":
                return X(h, 0, 0), X(h, 1, 2)
            if name == "K0":
                return X(h, 0, 1) - X(h, 0, 0), X(h, 0, 2) - X(h, 0, 3)
            return X(h, 1, 0) - X(h, 1, 1), X(h, 1, 3) - X(h, 1, 2)

        deep = {}
        for name, h in (("R0", 0), ("R1", 0), ("K0", 1), ("K1", 1)):
            (m0, n0), (m1, n1) = deep_rhs(name, h), deep_rhs(name, 1 - h)
            a = SLOT[name]
            p5 = mm(a + 4, 1, n1)
            p2 = mm(a + 1, 1, m0)
            p4 = mm(a + 3, 1, n0 - m0)
            p3 = mm(a + 2, 1, m1 - n1)
            if name[0] == "R":
                p5 = p5 + bias_ref[2 * int(name[1])]
                p2 = p2 + bias_ref[2 * int(name[1]) + 1]
            c01, c10, e00, e11 = p3 + p5, p2 + p4, p4 + p5, p2 + p3
            p1 = mm(a, 1, m0 - n1)
            p7 = mm(a + 6, 1, n0 - n1)
            p6 = mm(a + 5, 1, m1 - m0)
            deep[name, h] = [e00 + p1 + p7, c10]
            deep[name, 1 - h] = [c01, e11 - p1 + p6]
            at_point(next(points))

        def shallow(name, g, t):
            a = SLOT[name]
            both = mm(a, 1, jnp.concatenate([g[:64], t], axis=0))
            return [both + mm(a + 1, 1, g),
                    both + mm(a + 2, 1, jnp.concatenate([t, g[64:]], axis=0))]

        for h in range(2):
            for name, j, u in (("M1", 0, 0), ("N1", 1, 2)):
                y = mm(SLOT[name], 2, X(h, j, u) - X(h, 1 - j, u + 1))
                y = [y[:Q], y[Q:]]
                for i, jj, uu in ((0, j, u + 1), (1, 1 - j, u)):
                    d = shallow("D%d%d" % (i, jj), X(h, jj, uu) - X(h, 1 - jj, uu), X(h, jj, 4))
                    lanes = pl.ds(c % 2 * W + (2 * h + jj) * 128, 128)
                    for r in range(2):
                        v = deep["R%d" % i, h][r] + deep["K%d" % jj, h][r]
                        v = (v + y[r] if i == 0 else v - y[r]) + d[r]
                        v = v.astype(BF16).reshape(NU, 16, 128)
                        for first, part in ((0, v[:5]), (1, v[5:])):
                            g, o = divmod(NU * e + first, 2)
                            obuf[k, 2 * half + c // 2, g:g + part.shape[0],
                                 pl.ds(UR * o + 32 * i + 16 * r, 16), lanes] = part
                    at_point(next(points))

    n_steps = 2 * NP
    n_points = 8 * len(WRITE_POINTS)
    n_groups = 16 * (NP - 1)

    def next_group(step, t):
        return step * WRITE_RATE + (WRITE_BURST - (NP - 1) * WRITE_RATE + WRITE_RATE * t // n_points
                                    - WRITE_RATE * WRITE_START // n_points)

    assert next_group(n_steps, 0) >= n_groups
    assert all(2 * (r >> 4) + 2 <= i for i in range(NP - 1, n_steps)
               for r in range(next_group(i, 0), min(next_group(i + 1, 0), n_groups)))
    assert len(WRITE_LAST) <= 12 and all(t >= n_points // 2 for t in WRITE_LAST[8:])
    assert all(2 * (k - NI) + 1 < k - 1 for k in range(NI, NP))

    def start_dmas(step, q, point):
        if point in READ_POINTS:
            i0 = 16 * q + 4 * READ_POINTS.index(point)
            if i0 < 64:
                @pl.when(step == 0)
                def _():
                    for i in range(i0, i0 + 4):
                        start_read(0, 2 * (i >> 3) + (i & 1), 4 + ((i >> 1) & 3), xsem.at[4], i & 1)

            ahead, i0 = divmod(i0 + 64, 128)
            k = step + ahead
            for i1 in (i0, i0 + 2):
                @pl.when((k > 0) & (k < NP))
                def _():
                    for i in (i1, i1 + 1):
                        start_read(k, i >> 3, i & 7, xsem.at[4 + k], 0, hi=READ_SPLIT)
                        start_read(k, i >> 3, i & 7, xsem.at[4 + k], 1, lo=READ_SPLIT)

        if point in WRITE_POINTS:
            t = q * len(WRITE_POINTS) + WRITE_POINTS.index(point)
            for r in range(WRITE_BURST if t == WRITE_START else 0):
                @pl.when(step == NP - 1)
                def _():
                    start_row_group(r)

            for i in range(next_group(0, t + 1) - next_group(0, t)):
                r = next_group(step, t) + i

                @pl.when((r >= WRITE_BURST) & (r < n_groups))
                def _():
                    start_row_group(r)

            if t in WRITE_LAST:
                @pl.when(step == n_steps - 1)
                def _():
                    start_last_group(WRITE_LAST.index(t))

    @pl.loop(0, n_steps)
    def _(step):
        k, half = step >> 1, step & 1

        @pl.when(step == 1)
        def _():
            _wait_until_filled(xbuf.at[0, 4:8], xsem.at[4])

        @pl.when((k > 0) & (half == 0))
        def _():
            _wait_until_filled(xbuf.at[x_slot(k)], xsem.at[4 + k])

        for c in range(4):
            @pl.when(step == 0)
            def _():
                _wait_until_filled(xbuf.at[0, c], xsem.at[c])

            for e in range(2):
                compute_chunk(k, half, c, e, lambda point: start_dmas(step, 2 * c + e, point))

    for r in range(len(WRITE_LAST), 16):
        start_last_group(r)
    _wait_until_filled(obuf, osem.at[0])


@jax.jit
def pallas_standalone__structured_sparse_n_m__ragged_kernel(
    x: jax.Array,
    w: jax.Array,
    b: jax.Array,
):
    B, S, D = x.shape
    assert (B, S, D) == (16, 8 * W, NU * UR)
    xt = jnp.transpose(x, (0, 2, 1)).reshape(B // 2, NU, 2 * UR, S)
    out = pl.pallas_call(
        _kernel,
        in_specs=[pl.BlockSpec(memory_space=pl.ANY)] * 3,
        out_specs=pl.BlockSpec(memory_space=pl.ANY),
        out_shape=jax.ShapeDtypeStruct(xt.shape, x.dtype),
        scratch_shapes=[
            pltpu.VMEM((NI, S // W, NU, 2 * UR, W), BF16),
            pltpu.VMEM((B // 2, S // (2 * W), NU, 2 * UR, 2 * W), BF16),
            pltpu.VMEM((D, D), BF16),
            pltpu.VMEM((D,), BF16),
            pltpu.VMEM((NA, Q // 2, 128), I32),
            pltpu.VMEM((4, Q, 128), F32),
            pltpu.SemaphoreType.DMA((4 + B // 2,)),
            pltpu.SemaphoreType.DMA((1,)),
            pltpu.SemaphoreType.DMA((6,)),
        ],
        compiler_params=pltpu.CompilerParams(
            vmem_limit_bytes=127 * 1024 * 1024,
            disable_bounds_checks=True,
            disable_semaphore_checks=True,
            flags={"XLA_TPU_RESCHEDULE_DMA_DONES": True},
        ),
    )(xt, w, b)
    return jnp.transpose(out.reshape(B, D, S), (0, 2, 1))
```
